```python
import jax
import jax.numpy as jnp

def _softmax(x, axis=-1):
    return jax.nn.softmax(x, axis=axis)

def _gelu(x):
    return jax.nn.gelu(x, approximate=True)

def _silu(x):
    return jax.nn.silu(x)

def _sigmoid(x):
    return jax.nn.sigmoid(x)

def _layernorm(x, axis=-1, eps=1e-05):
    m = jnp.mean(x, axis=axis, keepdims=True)
    v = jnp.var(x, axis=axis, keepdims=True)
    return (x - m) / jnp.sqrt(v + eps)

def _scatter_add(tgt, idx, src, axis=0):
    return tgt.at[idx].add(src)

def _segment_sum(src, seg, n):
    return jax.ops.segment_sum(src, seg, n)

class _Rng:

    def __init__(self, key):
        self._k = key

    def _next(self):
        self._k, sub = jax.random.split(self._k)
        return sub

    def normal(self, shape):
        return jax.random.normal(self._next(), shape, dtype=jnp.bfloat16)

    def randint(self, lo, hi, shape):
        return jax.random.randint(self._next(), shape, lo, hi, dtype=jnp.int32)

    def uniform(self, shape, lo=0.0, hi=1.0):
        return jax.random.uniform(self._next(), shape, jnp.bfloat16, lo, hi)

    def permutation(self, n):
        return jax.random.permutation(self._next(), n)
kernel_name = 'adaLN_cond__sliding_block_cached__dense_activation_mish__decode'

def setup_inputs():
    _rng = _Rng(jax.random.key(int.from_bytes(__import__("os").urandom(4), "little")))
    _w = lambda a: (lambda t: t.astype(jnp.bfloat16) if jnp.issubdtype(t.dtype, jnp.floating) else t)(jnp.asarray(a))

    def _A_setup():
        B, Sq, D = (1, 1, 640)
        Hq, Hkv, Sk, Dh = (32, 32, 32768, 192)
        assert Hq % Hkv == 0, (Hq, Hkv)
        return {'x': _w((lambda *s: _rng.normal(s) * 0.05)(B, Sq, D)), 'k_cache': _w((lambda *s: _rng.normal(s) * 0.05)(B, Hkv, Sk, Dh)), 'v_cache': _w((lambda *s: _rng.normal(s) * 0.05)(B, Hkv, Sk, Dh)), 'wq': _w((lambda *s: _rng.normal(s) * 0.05)(D, Hq * Dh) * D ** (-0.5)), 'wo': _w((lambda *s: _rng.normal(s) * 0.05)(Hq * Dh, D) * (Hq * Dh) ** (-0.5))}
    _A_in = _A_setup()

    def _B_setup():
        B, S, D, F = (1, 1, 640, 1536)
        return {'x': _w((lambda *s: _rng.normal(s) * 0.05)(B, S, D)), 'w1': _w((lambda *s: _rng.normal(s) * 0.05)(D, F) * D ** (-0.5)), 'b1': _w((lambda *s: _rng.normal(s) * 0.05)(F)), 'w2': _w((lambda *s: _rng.normal(s) * 0.05)(F, D) * F ** (-0.5))}
    _B_in = _B_setup()
    return {'A_x': _A_in['x'], 'A_k_cache': _A_in['k_cache'], 'A_v_cache': _A_in['v_cache'], 'A_wq': _A_in['wq'], 'A_wo': _A_in['wo'], 'B_x': _B_in['x'], 'B_w1': _B_in['w1'], 'B_b1': _B_in['b1'], 'B_w2': _B_in['w2'], 'c': _w((lambda *s: _rng.normal(s) * 0.05)(1, 640)), 'w_mod': _w((lambda *s: _rng.normal(s) * 0.05)(640, 6 * 640) * 640 ** (-0.5))}

def reference(A_x, A_k_cache, A_v_cache, A_wq, A_wo, B_x, B_w1, B_b1, B_w2, c, w_mod):

    def _A_ref(x, k_cache, v_cache, wq, wo):
        B, Sq, D = x.shape
        Hq, Dh = (32, 192)
        Hkv, Sk = (k_cache.shape[1], k_cache.shape[2])
        W = min(4096, max(256, Sk // 4))
        rep = Hq // Hkv
        q = (lambda x, *d: x.transpose(*d))((x @ wq).reshape(B, Sq, Hq, Dh), 0, 2, 1, 3)
        k = jnp.repeat(k_cache[:, :, Sk - W:, :], rep, axis=1)
        v = jnp.repeat(v_cache[:, :, Sk - W:, :], rep, axis=1)
        scores = jnp.einsum('bhqd,bhkd->bhqk', q, k) * Dh ** (-0.5)
        p = _softmax(scores, axis=-1)
        o = jnp.einsum('bhqk,bhkd->bhqd', p, v)
        return (lambda x, *d: x.transpose(*d))(o, 0, 2, 1, 3).reshape(B, Sq, Hq * Dh) @ wo

    def _B_ref(x, w1, b1, w2):
        h = jnp.einsum('bsd,df->bsf', x, w1) + b1
        sp = jnp.log1p(jnp.exp(-jnp.abs(h))) + jnp.where(h > 0, h, jnp.zeros_like(h))
        act = h * jnp.tanh(sp)
        return jnp.einsum('bsf,fd->bsd', act, w2)
    x = A_x
    mod = (_silu(c) @ w_mod).reshape(c.shape[0], 6, 1, -1)
    sa, ca, ga, sb, cb, gb = (mod[:, 0].copy(), mod[:, 1].copy(), mod[:, 2].copy(), mod[:, 3].copy(), mod[:, 4].copy(), mod[:, 5].copy())
    h = _layernorm(x, axis=-1) * (1 + ca) + sa
    x = x + ga * _A_ref(h, A_k_cache, A_v_cache, A_wq, A_wo)
    h = _layernorm(x, axis=-1) * (1 + cb) + sb
    x = x + gb * _B_ref(h, B_w1, B_b1, B_w2)
    return x
```

```python
import functools

import jax
import jax.numpy as jnp
from jax import lax
import jax.experimental.pallas as pl
import jax.experimental.pallas.tpu as pltpu

D = 640
H = 32
DH = 192
F = 1536
PAIR = 2 * DH
NPAIR = H // 2
SUB = 8
LANE = 128
PIECE = 8
F32 = jnp.float32
BF16 = jnp.bfloat16

NSLOT = 3
QUEUE = (0, 1, 1, 1)
LAG = 25
LOOK = 80
W1_LOOK = 40
W2_LOOK = 35
PACE = 10
STEPS = 8
W2_LANES = 4
W2_MXU = (10, 10)
W2_VPU = (4, 3, 2, 1)


def _layernorm(x, eps=1e-5):
    m = jnp.mean(x, axis=-1, keepdims=True)
    d = x - m
    v = jnp.mean(d * d, axis=-1, keepdims=True)
    return d / jnp.sqrt(v + eps)


def _mish(u):
    softplus = jnp.log1p(jnp.exp(-jnp.abs(u))) + jnp.where(u > 0, u, 0.0)
    return u * jnp.tanh(softplus)


def _dot(a, b):
    return jnp.dot(a, b, preferred_element_type=F32)


def _num_pieces(ref):
    return ref.shape[0] * ref.shape[1] // (SUB * LANE * PIECE)


def _pieces(src, dst, sem, order):
    tiles = src.shape[1] // LANE
    out = []
    for q in order:
        t, end, rects = q * PIECE, (q + 1) * PIECE, []
        while t < end:
            r, c = divmod(t, tiles)
            n = min(tiles - c, end - t)
            idx = (pl.ds(r * SUB, SUB), pl.ds(c * LANE, n * LANE))
            rects.append(functools.partial(pltpu.make_async_copy, src.at[idx], dst.at[idx], sem))
            t += n
        out.append(rects)
    return out


def _matrix(src, dst, sem, jump):
    n = _num_pieces(src)
    return _pieces(src, dst, sem, [q for first in range(jump) for q in range(first, n, jump)])


class _Stream:
    def __init__(self, parts, fence, pos=0):
        self.ends = []
        pieces = []
        for i, part in enumerate(parts):
            pieces += [(i, piece) for piece in part]
            self.ends.append(len(pieces))
        queue = [QUEUE[n % len(QUEUE)] for n in range(len(pieces))]
        late = [(cp, 1, i) for (i, piece), q in zip(pieces, queue) if q for cp in piece]
        self.slots, taken = [], LAG
        for (i, piece), q in zip(pieces, queue):
            if q:
                self.slots.append(late[taken:taken + len(piece)])
                taken += len(piece)
            else:
                self.slots.append([(cp, 0, i) for cp in piece])
        self.slots[0] = late[:LAG] + self.slots[0]
        self.fence = fence
        self.pos = pos
        self.part = None

    def upto(self, n):
        while self.pos < min(n, len(self.slots)):
            for cp, queue, part in self.slots[self.pos]:
                if self.part not in (None, part):
                    self.fence()
                self.part = part
                cp().start(priority=queue)
            self.pos += 1

    def more(self, n):
        self.upto(self.pos + n)

    def past(self, part, look=LOOK):
        self.upto(self.ends[part] + look)


def _wait_all(buf, sem):
    pltpu.make_async_copy(buf, buf, sem).wait()


def _kernel(x_hbm, k_hbm, v_hbm, wq_hbm, wo_hbm, w1_hbm, b1_hbm, w2_hbm, c_hbm, wmod_hbm, o_ref,
            x_v, c_v, b1_v, wmod_v, wq_v, wo_v, w1_v, w2_v, kbuf, vbuf, q_s, s_s, acc_s, mod_s, act_s,
            sem_w, sem_kv, sem_fence):
    nc = kbuf.shape[1]
    col0 = k_hbm.shape[1] - nc
    rows = PAIR // SUB
    half = rows * nc // PIECE

    def kv_pieces(j, p):
        src, dst = ((k_hbm, kbuf), (v_hbm, vbuf))[j]
        slot = p % NSLOT
        return [[functools.partial(
            pltpu.make_async_copy, src.at[p * rows + r, pl.ds(col0 + c, PIECE)],
            dst.at[slot, pl.ds(c, PIECE), pl.ds(r * SUB, SUB), :], sem_kv.at[j, slot])]
            for first in range(2) for c in range(0, nc, PIECE) for r in range(first, rows, 2)]

    def fence():
        pl.semaphore_signal(sem_fence, 1)
        pl.semaphore_wait(sem_fence, 1)

    s_c, s_x, s_b1, s_wmod, s_wq, s_wo, s_w1, s_w2 = range(8)

    head = _Stream([
        _matrix(wmod_hbm, wmod_v, sem_w.at[s_wmod], 32),
        _matrix(wq_hbm, wq_v, sem_w.at[s_wq], 64),
        _matrix(wo_hbm, wo_v, sem_w.at[s_wo], 64),
        kv_pieces(0, 0), kv_pieces(1, 0)], fence)
    head.upto(1)
    small = [pltpu.make_async_copy(s, d, sem_w.at[i])
             for i, s, d in ((s_c, c_hbm, c_v), (s_x, x_hbm, x_v), (s_b1, b1_hbm, b1_v))]
    for cp in small:
        cp.start()
    head.past(0)
    for cp in small:
        cp.wait()
    _wait_all(wmod_v, sem_w.at[s_wmod])
    cf = c_v[...].astype(F32)
    silu_c = jnp.broadcast_to(cf * jax.nn.sigmoid(cf), (8, D)).astype(BF16)
    for i in range(6):
        mod_s[i] = _dot(silu_c, wmod_v[:, i * D:(i + 1) * D])
        head.more(48)
    x0 = jnp.broadcast_to(x_v[...].astype(F32), (8, D))
    h = (_layernorm(x0) * (1.0 + mod_s[1]) + mod_s[0]).astype(BF16)
    head.past(1)
    _wait_all(wq_v, sem_w.at[s_wq])
    row = lax.broadcasted_iota(jnp.int32, (8, PAIR), 0)
    col = lax.broadcasted_iota(jnp.int32, (8, PAIR), 1)
    own = jnp.logical_or(jnp.logical_and(row == 0, col < DH), jnp.logical_and(row == 1, col >= DH))
    for p in range(NPAIR):
        q_s[p] = jnp.where(own, _dot(h, wq_v[:, p * PAIR:(p + 1) * PAIR]), 0.0)
        head.more(24)
    head.past(2)
    _wait_all(wo_v, sem_w.at[s_wo])
    acc_s[...] = jnp.zeros(acc_s.shape, F32)
    head.past(3)

    def scores(p, stream, step):
        slot = p % NSLOT
        _wait_all(kbuf.at[slot], sem_kv.at[0, slot])
        q = q_s[p].astype(BF16)
        for i in range(STEPS):
            for c in range(i * nc // STEPS, (i + 1) * nc // STEPS):
                s_s[:, c * LANE:(c + 1) * LANE] = _dot(q, kbuf[slot, c]) * DH ** -0.5
            stream.more(step)
        s = s_s[...]
        e = jnp.exp(s - jnp.max(s, axis=-1, keepdims=True))
        s_s[...] = e
        return jnp.sum(e, axis=-1, keepdims=True)

    def values(p, denom, stream, step):
        slot = p % NSLOT
        _wait_all(vbuf.at[slot], sem_kv.at[1, slot])
        o = jnp.zeros((8, PAIR), F32)
        for i in range(STEPS):
            for c in range(i * nc // STEPS, (i + 1) * nc // STEPS):
                o += lax.dot_general(s_s[:, c * LANE:(c + 1) * LANE].astype(BF16), vbuf[slot, c],
                                     (((1,), (1,)), ((), ())), preferred_element_type=F32)
            stream.more(step)
        o = jnp.where(own, o / denom, 0.0).astype(BF16)
        r0 = p * PAIR
        if not isinstance(r0, int):
            r0 = pl.multiple_of(r0, PAIR)
        acc_s[...] += _dot(o, wo_v[pl.ds(r0, PAIR), :])

    def body(p, carry):
        stream = _Stream([kv_pieces(1, p), kv_pieces(0, p + 1), kv_pieces(1, p + 1)], fence, LOOK)
        denom = scores(p, stream, half // (STEPS + 1))
        stream.past(0)
        values(p, denom, stream, half // (STEPS + 1))
        stream.past(1)
        return carry

    lax.fori_loop(0, NPAIR - 1, body, 0)

    per_lane = _num_pieces(w2_v) // W2_LANES
    groups, first = [], 0
    for n in W2_MXU + W2_VPU:
        groups.append([l * per_lane + q for q in range(first, first + n) for l in range(W2_LANES)])
        first += n
    assert first == per_lane
    w2_parts = [_pieces(w2_hbm, w2_v, sem_w.at[s_w2 + i], g) for i, g in enumerate(groups)]
    tail = _Stream([kv_pieces(1, NPAIR - 1), _matrix(w1_hbm, w1_v, sem_w.at[s_w1], 32),
                    [piece for part in w2_parts for piece in part]], fence, LOOK)
    denom = scores(NPAIR - 1, tail, (half - 20) // (STEPS + 1))
    tail.past(0, LOOK - 20)
    values(NPAIR - 1, denom, tail, PACE)

    att = jnp.broadcast_to(jnp.sum(acc_s[...], axis=0, keepdims=True), (8, D))
    x1 = x0 + mod_s[2] * att
    h2 = (_layernorm(x1) * (1.0 + mod_s[4]) + mod_s[3]).astype(BF16)
    b1 = b1_v[...].astype(F32)
    tail.past(1, W1_LOOK)
    _wait_all(w1_v, sem_w.at[s_w1])
    width = F // W2_LANES
    acts = []
    for c0 in range(0, F, width):
        bias = jnp.concatenate([jnp.broadcast_to(b1[t:t + 1, :], (8, LANE))
                                for t in range(c0 // LANE, (c0 + width) // LANE)], axis=1)
        acts.append(_mish(_dot(h2, w1_v[:, c0:c0 + width]) + bias).astype(BF16))
        tail.more(PACE)
    act = jnp.concatenate(acts, axis=1)
    for l in range(W2_LANES):
        for c0 in range(l * width + len(W2_MXU) * LANE, (l + 1) * width, LANE):
            act_s[c0:c0 + LANE, :] = jnp.broadcast_to(act[:1, c0:c0 + LANE].astype(F32), (LANE, LANE)).T

    y = jnp.zeros((8, D), F32)
    done = tail.ends[1]
    for i in range(len(W2_MXU)):
        done += len(groups[i])
        tail.upto(done + W2_LOOK)
        starts = [l * width + i * LANE for l in range(W2_LANES)]
        for r in starts:
            _wait_all(w2_v.at[pl.ds(r, LANE)], sem_w.at[s_w2 + i])
        for r in starts:
            y += _dot(act[:, r:r + LANE], w2_v[r:r + LANE, :])
            acc_s[...] = y
            tail.more(2)
    tail.past(2)
    gate = mod_s[5]
    partial = x1 + gate * y
    acc = [jnp.zeros((SUB, LANE), F32)] * (D // LANE)
    for i in range(len(W2_MXU), len(groups)):
        for piece in w2_parts[i]:
            for cp in piece:
                cp().wait()
        for q in groups[i]:
            for t in range(q * PIECE, (q + 1) * PIECE):
                r, c = divmod(t, D // LANE)
                w = w2_v[r * SUB:(r + 1) * SUB, c * LANE:(c + 1) * LANE].astype(F32)
                acc[c] = acc[c] + w * act_s[r * SUB:(r + 1) * SUB, :]
        acc_s[...] = jnp.concatenate(acc, axis=1)
    y = jnp.sum(jnp.concatenate(acc, axis=1), axis=0, keepdims=True)
    o_ref[...] = (partial[0:1] + gate[0:1] * y).astype(o_ref.dtype)


def _tiles(cache):
    t = jnp.swapaxes(cache, 2, 3).reshape(H * DH // SUB, SUB, cache.shape[2] // LANE, LANE)
    return t.transpose(0, 2, 1, 3)


@jax.jit
def pallas_adaLN_cond__sliding_block_cached__dense_activation_mish__decode_kernel(
    A_x: jax.Array,
    A_k_cache: jax.Array,
    A_v_cache: jax.Array,
    A_wq: jax.Array,
    A_wo: jax.Array,
    B_x: jax.Array,
    B_w1: jax.Array,
    B_b1: jax.Array,
    B_w2: jax.Array,
    c: jax.Array,
    w_mod: jax.Array,
):
    del B_x
    window = min(4096, max(256, A_k_cache.shape[2] // 4))
    hbm = pl.BlockSpec(memory_space=pltpu.HBM)
    out = pl.pallas_call(
        _kernel,
        out_shape=jax.ShapeDtypeStruct((1, D), A_x.dtype),
        in_specs=[hbm] * 10,
        out_specs=pl.BlockSpec(memory_space=pltpu.VMEM),
        scratch_shapes=[
            pltpu.VMEM((1, D), BF16),
            pltpu.VMEM((1, D), BF16),
            pltpu.VMEM((F // LANE, LANE), BF16),
            pltpu.VMEM((D, 6 * D), BF16),
            pltpu.VMEM((D, H * DH), BF16),
            pltpu.VMEM((H * DH, D), BF16),
            pltpu.VMEM((D, F), BF16),
            pltpu.VMEM((F, D), BF16),
            pltpu.VMEM((NSLOT, window // LANE, PAIR, LANE), BF16),
            pltpu.VMEM((NSLOT, window // LANE, PAIR, LANE), BF16),
            pltpu.VMEM((NPAIR, 8, PAIR), F32),
            pltpu.VMEM((8, window), F32),
            pltpu.VMEM((8, D), F32),
            pltpu.VMEM((6, 8, D), F32),
            pltpu.VMEM((F, LANE), F32),
            pltpu.SemaphoreType.DMA((7 + len(W2_MXU) + len(W2_VPU),)),
            pltpu.SemaphoreType.DMA((2, NSLOT)),
            pltpu.SemaphoreType.REGULAR,
        ],
        compiler_params=pltpu.CompilerParams(
            vmem_limit_bytes=64 * 2**20,
            disable_semaphore_checks=True,
        ),
        name="adaln_attn_mlp_decode",
    )(A_x.reshape(1, D), _tiles(A_k_cache), _tiles(A_v_cache), A_wq, A_wo, B_w1,
      B_b1.reshape(F // LANE, LANE), B_w2, c, w_mod)
    return out.reshape(A_x.shape)
```

```python
import functools

import jax
import jax.numpy as jnp
from jax import lax
import jax.experimental.pallas as pl
import jax.experimental.pallas.tpu as pltpu

D = 640
H = 32
DH = 192
F = 1536
PAIR = 2 * DH
NPAIR = H // 2
SUB = 8
LANE = 128
PIECE = 8
F32 = jnp.float32
BF16 = jnp.bfloat16

NSLOT = 3
QUEUE = (0, 1, 1, 1)
LAG = 25
LOOK = 80
W1_LOOK = 40
W2_LOOK = 35
PACE = 10
STEPS = 8
W2_LANES = 4
W2_MXU = (10, 10)
W2_VPU = (4, 3, 2, 1)


def _layernorm(x, eps=1e-5):
    m = jnp.mean(x, axis=-1, keepdims=True)
    d = x - m
    v = jnp.mean(d * d, axis=-1, keepdims=True)
    return d / jnp.sqrt(v + eps)


def _mish(u):
    softplus = jnp.log1p(jnp.exp(-jnp.abs(u))) + jnp.where(u > 0, u, 0.0)
    return u * jnp.tanh(softplus)


def _dot(a, b):
    return jnp.dot(a, b, preferred_element_type=F32)


def _num_pieces(ref):
    return ref.shape[0] * ref.shape[1] // (SUB * LANE * PIECE)


def _pieces(src, dst, sem, order):
    tiles = src.shape[1] // LANE
    out = []
    for q in order:
        t, end, rects = q * PIECE, (q + 1) * PIECE, []
        while t < end:
            r, c = divmod(t, tiles)
            n = min(tiles - c, end - t)
            idx = (pl.ds(r * SUB, SUB), pl.ds(c * LANE, n * LANE))
            rects.append(functools.partial(pltpu.make_async_copy, src.at[idx], dst.at[idx], sem))
            t += n
        out.append(rects)
    return out


def _matrix(src, dst, sem, jump):
    n = _num_pieces(src)
    return _pieces(src, dst, sem, [q for first in range(jump) for q in range(first, n, jump)])


class _Stream:
    def __init__(self, parts, fence, pos=0):
        self.ends = []
        pieces = []
        for i, part in enumerate(parts):
            pieces += [(i, piece) for piece in part]
            self.ends.append(len(pieces))
        queue = [QUEUE[n % len(QUEUE)] for n in range(len(pieces))]
        late = [(cp, 1, i) for (i, piece), q in zip(pieces, queue) if q for cp in piece]
        self.slots, taken = [], LAG
        for (i, piece), q in zip(pieces, queue):
            if q:
                self.slots.append(late[taken:taken + len(piece)])
                taken += len(piece)
            else:
                self.slots.append([(cp, 0, i) for cp in piece])
        self.slots[0] = late[:LAG] + self.slots[0]
        self.fence = fence
        self.pos = pos
        self.part = None

    def upto(self, n):
        while self.pos < min(n, len(self.slots)):
            for cp, queue, part in self.slots[self.pos]:
                if self.part not in (None, part):
                    self.fence()
                self.part = part
                cp().start(priority=queue)
            self.pos += 1

    def more(self, n):
        self.upto(self.pos + n)

    def past(self, part, look=LOOK):
        self.upto(self.ends[part] + look)


def _wait_all(buf, sem):
    pltpu.make_async_copy(buf, buf, sem).wait()


def _wait_pieces(pieces):
    for piece in pieces:
        for cp in piece:
            cp().wait()


def _kernel(x_hbm, k_hbm, v_hbm, wq_hbm, wo_hbm, w1_hbm, b1_hbm, w2_hbm, c_hbm, wmod_hbm, o_ref,
            x_v, c_v, b1_v, wmod_v, wq_v, wo_v, w1_v, w2_v, kbuf, vbuf, q_s, s_s, acc_s, mod_s, act_s,
            sem_w, sem_kv, sem_fence):
    nc = kbuf.shape[1]
    col0 = k_hbm.shape[1] - nc
    rows = PAIR // SUB
    half = rows * nc // PIECE

    def kv_pieces(j, p):
        src, dst = ((k_hbm, kbuf), (v_hbm, vbuf))[j]
        slot = p % NSLOT
        return [[functools.partial(
            pltpu.make_async_copy, src.at[p * rows + r, pl.ds(col0 + c, PIECE)],
            dst.at[slot, pl.ds(c, PIECE), pl.ds(r * SUB, SUB), :], sem_kv.at[j, slot])]
            for r0 in (0, rows // 2) for first in (r0, r0 + 1) for c in range(0, nc, PIECE)
            for r in range(first, r0 + rows // 2, 2)]

    def fence():
        pl.semaphore_signal(sem_fence, 1)
        pl.semaphore_wait(sem_fence, 1)

    s_c, s_x, s_b1, s_wmod, s_wq, s_wo, s_w1, s_w2 = range(8)

    head = _Stream([
        _matrix(wmod_hbm, wmod_v, sem_w.at[s_wmod], 32),
        _matrix(wq_hbm, wq_v, sem_w.at[s_wq], 64),
        _matrix(wo_hbm, wo_v, sem_w.at[s_wo], 64),
        kv_pieces(0, 0), kv_pieces(1, 0)], fence)
    head.upto(1)
    small = [pltpu.make_async_copy(s, d, sem_w.at[i])
             for i, s, d in ((s_c, c_hbm, c_v), (s_x, x_hbm, x_v), (s_b1, b1_hbm, b1_v))]
    for cp in small:
        cp.start()
    head.past(0)
    for cp in small:
        cp.wait()
    _wait_all(wmod_v, sem_w.at[s_wmod])
    cf = c_v[...].astype(F32)
    silu_c = jnp.broadcast_to(cf * jax.nn.sigmoid(cf), (8, D)).astype(BF16)
    for i in range(6):
        mod_s[i] = _dot(silu_c, wmod_v[:, i * D:(i + 1) * D])
        head.more(48)
    x0 = jnp.broadcast_to(x_v[...].astype(F32), (8, D))
    h = (_layernorm(x0) * (1.0 + mod_s[1]) + mod_s[0]).astype(BF16)
    head.past(1)
    _wait_all(wq_v, sem_w.at[s_wq])
    row = lax.broadcasted_iota(jnp.int32, (8, PAIR), 0)
    col = lax.broadcasted_iota(jnp.int32, (8, PAIR), 1)
    own = jnp.logical_or(jnp.logical_and(row == 0, col < DH), jnp.logical_and(row == 1, col >= DH))
    for p in range(NPAIR):
        q_s[p] = jnp.where(own, _dot(h, wq_v[:, p * PAIR:(p + 1) * PAIR]), 0.0)
        head.more(24)
    head.past(2)
    _wait_all(wo_v, sem_w.at[s_wo])
    acc_s[...] = jnp.zeros(acc_s.shape, F32)
    head.past(3)

    def scores(p, stream, step):
        slot = p % NSLOT
        _wait_all(kbuf.at[slot], sem_kv.at[0, slot])
        q = q_s[p].astype(BF16)
        for i in range(STEPS):
            for c in range(i * nc // STEPS, (i + 1) * nc // STEPS):
                s_s[:, c * LANE:(c + 1) * LANE] = _dot(q, kbuf[slot, c]) * DH ** -0.5
            stream.more(step)
        s = s_s[...]
        e = jnp.exp(s - jnp.max(s, axis=-1, keepdims=True))
        s_s[...] = e
        return jnp.sum(e, axis=-1, keepdims=True)

    def values(p, denom, stream, step):
        slot = p % NSLOT
        _wait_all(vbuf.at[slot], sem_kv.at[1, slot])
        o = jnp.zeros((8, PAIR), F32)
        for i in range(STEPS):
            for c in range(i * nc // STEPS, (i + 1) * nc // STEPS):
                o += lax.dot_general(s_s[:, c * LANE:(c + 1) * LANE].astype(BF16), vbuf[slot, c],
                                     (((1,), (1,)), ((), ())), preferred_element_type=F32)
            stream.more(step)
        o = jnp.where(own, o / denom, 0.0).astype(BF16)
        r0 = p * PAIR
        if not isinstance(r0, int):
            r0 = pl.multiple_of(r0, PAIR)
        acc_s[...] += _dot(o, wo_v[pl.ds(r0, PAIR), :])

    def body(p, carry):
        stream = _Stream([kv_pieces(1, p), kv_pieces(0, p + 1), kv_pieces(1, p + 1)], fence, LOOK)
        denom = scores(p, stream, half // (STEPS + 1))
        stream.past(0)
        values(p, denom, stream, half // (STEPS + 1))
        stream.past(1)
        return carry

    lax.fori_loop(0, NPAIR - 1, body, 0)

    per_lane = _num_pieces(w2_v) // W2_LANES
    groups, first = [], 0
    for n in W2_MXU + W2_VPU:
        groups.append([l * per_lane + q for q in range(first, first + n) for l in range(W2_LANES)])
        first += n
    assert first == per_lane
    w2_parts = [_pieces(w2_hbm, w2_v, sem_w.at[s_w2 + i], g) for i, g in enumerate(groups)]
    tail = _Stream([kv_pieces(1, NPAIR - 1), _matrix(w1_hbm, w1_v, sem_w.at[s_w1], 32),
                    [piece for part in w2_parts for piece in part]], fence, LOOK)
    denom = scores(NPAIR - 1, tail, (half - 20) // (STEPS + 1))
    tail.past(0, LOOK - 20)
    values(NPAIR - 1, denom, tail, PACE)

    att = jnp.broadcast_to(jnp.sum(acc_s[...], axis=0, keepdims=True), (8, D))
    x1 = x0 + mod_s[2] * att
    h2 = (_layernorm(x1) * (1.0 + mod_s[4]) + mod_s[3]).astype(BF16)
    b1 = b1_v[...].astype(F32)
    tail.past(1, W1_LOOK)
    _wait_all(w1_v, sem_w.at[s_w1])
    width = F // W2_LANES
    acts = []
    for c0 in range(0, F, width):
        bias = jnp.concatenate([jnp.broadcast_to(b1[t:t + 1, :], (8, LANE))
                                for t in range(c0 // LANE, (c0 + width) // LANE)], axis=1)
        acts.append(_mish(_dot(h2, w1_v[:, c0:c0 + width]) + bias).astype(BF16))
        tail.more(PACE)
    act = jnp.concatenate(acts, axis=1)
    for l in range(W2_LANES):
        for c0 in range(l * width + len(W2_MXU) * LANE, (l + 1) * width, LANE):
            act_s[c0:c0 + LANE, :] = jnp.broadcast_to(act[:1, c0:c0 + LANE].astype(F32), (LANE, LANE)).T

    y = jnp.zeros((8, D), F32)
    done = tail.ends[1]
    for i in range(len(W2_MXU)):
        done += len(groups[i])
        tail.upto(done + W2_LOOK)
        _wait_pieces(w2_parts[i])
        for r in range(i * LANE, F, width):
            y += _dot(act[:, r:r + LANE], w2_v[r:r + LANE, :])
            acc_s[...] = y
            tail.more(2)
    tail.past(2)
    gate = mod_s[5]
    partial = x1 + gate * y
    acc = [jnp.zeros((SUB, LANE), F32)] * (D // LANE)
    for i in range(len(W2_MXU), len(groups)):
        _wait_pieces(w2_parts[i])
        for q in groups[i]:
            for t in range(q * PIECE, (q + 1) * PIECE):
                r, c = divmod(t, D // LANE)
                w = w2_v[r * SUB:(r + 1) * SUB, c * LANE:(c + 1) * LANE].astype(F32)
                acc[c] = acc[c] + w * act_s[r * SUB:(r + 1) * SUB, :]
        acc_s[...] = jnp.concatenate(acc, axis=1)
    y = jnp.sum(jnp.concatenate(acc, axis=1), axis=0, keepdims=True)
    o_ref[...] = (partial[0:1] + gate[0:1] * y).astype(o_ref.dtype)


def _tiles(cache):
    t = jnp.swapaxes(cache, 2, 3).reshape(H * DH // SUB, SUB, cache.shape[2] // LANE, LANE)
    return t.transpose(0, 2, 1, 3)


@jax.jit
def pallas_adaLN_cond__sliding_block_cached__dense_activation_mish__decode_kernel(
    A_x: jax.Array,
    A_k_cache: jax.Array,
    A_v_cache: jax.Array,
    A_wq: jax.Array,
    A_wo: jax.Array,
    B_x: jax.Array,
    B_w1: jax.Array,
    B_b1: jax.Array,
    B_w2: jax.Array,
    c: jax.Array,
    w_mod: jax.Array,
):
    del B_x
    window = min(4096, max(256, A_k_cache.shape[2] // 4))
    hbm = pl.BlockSpec(memory_space=pltpu.HBM)
    out = pl.pallas_call(
        _kernel,
        out_shape=jax.ShapeDtypeStruct((1, D), A_x.dtype),
        in_specs=[hbm] * 10,
        out_specs=pl.BlockSpec(memory_space=pltpu.VMEM),
        scratch_shapes=[
            pltpu.VMEM((1, D), BF16),
            pltpu.VMEM((1, D), BF16),
            pltpu.VMEM((F // LANE, LANE), BF16),
            pltpu.VMEM((D, 6 * D), BF16),
            pltpu.VMEM((D, H * DH), BF16),
            pltpu.VMEM((H * DH, D), BF16),
            pltpu.VMEM((D, F), BF16),
            pltpu.VMEM((F, D), BF16),
            pltpu.VMEM((NSLOT, window // LANE, PAIR, LANE), BF16),
            pltpu.VMEM((NSLOT, window // LANE, PAIR, LANE), BF16),
            pltpu.VMEM((NPAIR, 8, PAIR), F32),
            pltpu.VMEM((8, window), F32),
            pltpu.VMEM((8, D), F32),
            pltpu.VMEM((6, 8, D), F32),
            pltpu.VMEM((F, LANE), F32),
            pltpu.SemaphoreType.DMA((7 + len(W2_MXU) + len(W2_VPU),)),
            pltpu.SemaphoreType.DMA((2, NSLOT)),
            pltpu.SemaphoreType.REGULAR,
        ],
        compiler_params=pltpu.CompilerParams(
            vmem_limit_bytes=64 * 2**20,
            disable_semaphore_checks=True,
        ),
        name="adaln_attn_mlp_decode",
    )(A_x.reshape(1, D), _tiles(A_k_cache), _tiles(A_v_cache), A_wq, A_wo, B_w1,
      B_b1.reshape(F // LANE, LANE), B_w2, c, w_mod)
    return out.reshape(A_x.shape)
```

```python
import functools

import jax
import jax.numpy as jnp
from jax import lax
import jax.experimental.pallas as pl
import jax.experimental.pallas.tpu as pltpu

D = 640
H = 32
DH = 192
F = 1536
PAIR = 2 * DH
NPAIR = H // 2
SUB = 8
LANE = 128
PIECE = 8
F32 = jnp.float32
BF16 = jnp.bfloat16

NSLOT = 3
SHIFT = 4
QUEUE = (0, 1, 1, 1)
LAG = 25
LOOK = 80
W1_LOOK = 40
W2_LOOK = 35
PACE = 10
STEPS = 8
W2_LANES = 4
W2_MXU = (10, 10)
W2_VPU = (4, 3, 2, 1)


def _layernorm(x, eps=1e-5):
    m = jnp.mean(x, axis=-1, keepdims=True)
    d = x - m
    v = jnp.mean(d * d, axis=-1, keepdims=True)
    return d / jnp.sqrt(v + eps)


def _mish(u):
    softplus = jnp.log1p(jnp.exp(-jnp.abs(u))) + jnp.where(u > 0, u, 0.0)
    return u * jnp.tanh(softplus)


def _dot(a, b):
    return jnp.dot(a, b, preferred_element_type=F32)


def _num_pieces(ref):
    return ref.shape[0] * ref.shape[1] // (SUB * LANE * PIECE)


def _pieces(src, dst, sem, order):
    tiles = src.shape[1] // LANE
    out = []
    for q in order:
        t, end, rects = q * PIECE, (q + 1) * PIECE, []
        while t < end:
            r, c = divmod(t, tiles)
            n = min(tiles - c, end - t)
            idx = (pl.ds(r * SUB, SUB), pl.ds(c * LANE, n * LANE))
            rects.append(functools.partial(pltpu.make_async_copy, src.at[idx], dst.at[idx], sem))
            t += n
        out.append(rects)
    return out


def _matrix(src, dst, sem, jump):
    n = _num_pieces(src)
    return _pieces(src, dst, sem, [q for first in range(jump) for q in range(first, n, jump)])


class _Stream:
    def __init__(self, parts, fence, pos=0):
        self.ends = []
        pieces = []
        for i, part in enumerate(parts):
            pieces += [(i, piece) for piece in part]
            self.ends.append(len(pieces))
        queue = [QUEUE[n % len(QUEUE)] for n in range(len(pieces))]
        late = [(cp, 1, i) for (i, piece), q in zip(pieces, queue) if q for cp in piece]
        self.slots, taken = [], LAG
        for (i, piece), q in zip(pieces, queue):
            if q:
                self.slots.append(late[taken:taken + len(piece)])
                taken += len(piece)
            else:
                self.slots.append([(cp, 0, i) for cp in piece])
        self.slots[0] = late[:LAG] + self.slots[0]
        self.fence = fence
        self.pos = pos
        self.part = None

    def upto(self, n):
        while self.pos < min(n, len(self.slots)):
            for cp, queue, part in self.slots[self.pos]:
                if self.part not in (None, part):
                    self.fence()
                self.part = part
                cp().start(priority=queue)
            self.pos += 1

    def more(self, n):
        self.upto(self.pos + n)

    def past(self, part, look=LOOK):
        self.upto(self.ends[part] + look)


def _wait_all(buf, sem):
    pltpu.make_async_copy(buf, buf, sem).wait()


def _wait_pieces(pieces):
    for piece in pieces:
        for cp in piece:
            cp().wait()


def _kernel(x_hbm, k_hbm, v_hbm, wq_hbm, wo_hbm, w1_hbm, b1_hbm, w2_hbm, c_hbm, wmod_hbm, o_ref,
            x_v, c_v, b1_v, wmod_v, wq_v, wo_v, w1_v, w2_v, kbuf, vbuf, q_s, s_s, acc_s, mod_s, act_s,
            sem_w, sem_kv, sem_fence):
    nc = kbuf.shape[1]
    col0 = k_hbm.shape[1] - nc
    rows = PAIR // SUB
    half = rows * nc // PIECE

    def kv_piece(j, p, r, c):
        src, dst = ((k_hbm, kbuf), (v_hbm, vbuf))[j]
        slot = (p + r // rows) % NSLOT
        return [functools.partial(
            pltpu.make_async_copy, src.at[p * rows + r, pl.ds(col0 + c, PIECE)],
            dst.at[slot, pl.ds(c, PIECE), pl.ds(r % rows * SUB, SUB), :], sem_kv.at[j, slot])]

    def kv_pieces(j, p):
        last = isinstance(p, int) and p == NPAIR - 1
        blocks = (SHIFT, SHIFT + rows // 2), (SHIFT + rows // 2, rows if last else SHIFT + rows)
        return [kv_piece(j, p, r, c) for lo, hi in blocks for first in (lo, lo + 1)
                for c in range(0, nc, PIECE) for r in range(first, hi, 2)]

    def fence():
        pl.semaphore_signal(sem_fence, 1)
        pl.semaphore_wait(sem_fence, 1)

    s_c, s_x, s_b1, s_wmod, s_wq, s_wo, s_w1, s_w2 = range(8)

    head = _Stream([
        _matrix(wmod_hbm, wmod_v, sem_w.at[s_wmod], 32),
        _matrix(wq_hbm, wq_v, sem_w.at[s_wq], 64),
        _matrix(wo_hbm, wo_v, sem_w.at[s_wo], 64),
        *[[kv_piece(j, 0, r, c) for r in range(SHIFT)] for c in range(0, nc, PIECE) for j in range(2)],
        kv_pieces(0, 0), kv_pieces(1, 0)], fence)
    head.upto(1)
    small = [pltpu.make_async_copy(s, d, sem_w.at[i])
             for i, s, d in ((s_c, c_hbm, c_v), (s_x, x_hbm, x_v), (s_b1, b1_hbm, b1_v))]
    for cp in small:
        cp.start()
    head.past(0)
    for cp in small:
        cp.wait()
    _wait_all(wmod_v, sem_w.at[s_wmod])
    cf = c_v[...].astype(F32)
    silu_c = jnp.broadcast_to(cf * jax.nn.sigmoid(cf), (8, D)).astype(BF16)
    for i in range(6):
        mod_s[i] = _dot(silu_c, wmod_v[:, i * D:(i + 1) * D])
        head.more(48)
    x0 = jnp.broadcast_to(x_v[...].astype(F32), (8, D))
    h = (_layernorm(x0) * (1.0 + mod_s[1]) + mod_s[0]).astype(BF16)
    head.past(1)
    _wait_all(wq_v, sem_w.at[s_wq])
    row = lax.broadcasted_iota(jnp.int32, (8, PAIR), 0)
    col = lax.broadcasted_iota(jnp.int32, (8, PAIR), 1)
    own = jnp.logical_or(jnp.logical_and(row == 0, col < DH), jnp.logical_and(row == 1, col >= DH))
    for p in range(NPAIR):
        q_s[p] = jnp.where(own, _dot(h, wq_v[:, p * PAIR:(p + 1) * PAIR]), 0.0)
        head.more(24)
    head.past(2)
    _wait_all(wo_v, sem_w.at[s_wo])
    acc_s[...] = jnp.zeros(acc_s.shape, F32)
    head.past(-2)

    def scores(p, stream, step):
        slot = p % NSLOT
        _wait_all(kbuf.at[slot], sem_kv.at[0, slot])
        q = q_s[p].astype(BF16)
        for i in range(STEPS):
            for c in range(i * nc // STEPS, (i + 1) * nc // STEPS):
                s_s[:, c * LANE:(c + 1) * LANE] = _dot(q, kbuf[slot, c]) * DH ** -0.5
            stream.more(step)
        s = s_s[...]
        e = jnp.exp(s - jnp.max(s, axis=-1, keepdims=True))
        s_s[...] = e
        return jnp.sum(e, axis=-1, keepdims=True)

    def values(p, denom, stream, step):
        slot = p % NSLOT
        _wait_all(vbuf.at[slot], sem_kv.at[1, slot])
        o = jnp.zeros((8, PAIR), F32)
        for i in range(STEPS):
            for c in range(i * nc // STEPS, (i + 1) * nc // STEPS):
                o += lax.dot_general(s_s[:, c * LANE:(c + 1) * LANE].astype(BF16), vbuf[slot, c],
                                     (((1,), (1,)), ((), ())), preferred_element_type=F32)
            stream.more(step)
        o = jnp.where(own, o / denom, 0.0).astype(BF16)
        r0 = p * PAIR
        if not isinstance(r0, int):
            r0 = pl.multiple_of(r0, PAIR)
        acc_s[...] += _dot(o, wo_v[pl.ds(r0, PAIR), :])

    def body(p, carry):
        stream = _Stream([kv_pieces(1, p), kv_pieces(0, p + 1), kv_pieces(1, p + 1)], fence, LOOK)
        denom = scores(p, stream, half // (STEPS + 1))
        stream.past(0)
        values(p, denom, stream, half // (STEPS + 1))
        stream.past(1)
        return carry

    lax.fori_loop(0, NPAIR - 2, body, 0)

    per_lane = _num_pieces(w2_v) // W2_LANES
    groups, first = [], 0
    for n in W2_MXU + W2_VPU:
        groups.append([l * per_lane + q for q in range(first, first + n) for l in range(W2_LANES)])
        first += n
    assert first == per_lane
    w2_parts = [_pieces(w2_hbm, w2_v, sem_w.at[s_w2 + i], g) for i, g in enumerate(groups)]
    tail = _Stream([kv_pieces(1, NPAIR - 2), kv_pieces(0, NPAIR - 1), kv_pieces(1, NPAIR - 1),
                    _matrix(w1_hbm, w1_v, sem_w.at[s_w1], 32),
                    [piece for part in w2_parts for piece in part]], fence, LOOK)
    denom = scores(NPAIR - 2, tail, half // (STEPS + 1))
    tail.past(0)
    values(NPAIR - 2, denom, tail, half // (STEPS + 2))
    tail.past(1)
    denom = scores(NPAIR - 1, tail, half // (STEPS + 4))
    tail.past(2, LOOK - 20)
    values(NPAIR - 1, denom, tail, PACE)

    att = jnp.broadcast_to(jnp.sum(acc_s[...], axis=0, keepdims=True), (8, D))
    x1 = x0 + mod_s[2] * att
    h2 = (_layernorm(x1) * (1.0 + mod_s[4]) + mod_s[3]).astype(BF16)
    b1 = b1_v[...].astype(F32)
    tail.past(3, W1_LOOK)
    _wait_all(w1_v, sem_w.at[s_w1])
    width = F // W2_LANES
    acts = []
    for c0 in range(0, F, width):
        bias = jnp.concatenate([jnp.broadcast_to(b1[t:t + 1, :], (8, LANE))
                                for t in range(c0 // LANE, (c0 + width) // LANE)], axis=1)
        acts.append(_mish(_dot(h2, w1_v[:, c0:c0 + width]) + bias).astype(BF16))
        tail.more(PACE)
    act = jnp.concatenate(acts, axis=1)
    for l in range(W2_LANES):
        for c0 in range(l * width + len(W2_MXU) * LANE, (l + 1) * width, LANE):
            act_s[c0:c0 + LANE, :] = jnp.broadcast_to(act[:1, c0:c0 + LANE].astype(F32), (LANE, LANE)).T

    y = jnp.zeros((8, D), F32)
    done = tail.ends[3]
    for i in range(len(W2_MXU)):
        done += len(groups[i])
        tail.upto(done + W2_LOOK)
        _wait_pieces(w2_parts[i])
        for r in range(i * LANE, F, width):
            y += _dot(act[:, r:r + LANE], w2_v[r:r + LANE, :])
            acc_s[...] = y
            tail.more(2)
    tail.past(4)
    gate = mod_s[5]
    partial = x1 + gate * y
    acc = [jnp.zeros((SUB, LANE), F32)] * (D // LANE)
    for i in range(len(W2_MXU), len(groups)):
        _wait_pieces(w2_parts[i])
        for q in groups[i]:
            for t in range(q * PIECE, (q + 1) * PIECE):
                r, c = divmod(t, D // LANE)
                w = w2_v[r * SUB:(r + 1) * SUB, c * LANE:(c + 1) * LANE].astype(F32)
                acc[c] = acc[c] + w * act_s[r * SUB:(r + 1) * SUB, :]
        acc_s[...] = jnp.concatenate(acc, axis=1)
    y = jnp.sum(jnp.concatenate(acc, axis=1), axis=0, keepdims=True)
    o_ref[...] = (partial[0:1] + gate[0:1] * y).astype(o_ref.dtype)


def _tiles(cache):
    t = jnp.swapaxes(cache, 2, 3).reshape(H * DH // SUB, SUB, cache.shape[2] // LANE, LANE)
    return t.transpose(0, 2, 1, 3)


@jax.jit
def pallas_adaLN_cond__sliding_block_cached__dense_activation_mish__decode_kernel(
    A_x: jax.Array,
    A_k_cache: jax.Array,
    A_v_cache: jax.Array,
    A_wq: jax.Array,
    A_wo: jax.Array,
    B_x: jax.Array,
    B_w1: jax.Array,
    B_b1: jax.Array,
    B_w2: jax.Array,
    c: jax.Array,
    w_mod: jax.Array,
):
    del B_x
    window = min(4096, max(256, A_k_cache.shape[2] // 4))
    hbm = pl.BlockSpec(memory_space=pltpu.HBM)
    out = pl.pallas_call(
        _kernel,
        out_shape=jax.ShapeDtypeStruct((1, D), A_x.dtype),
        in_specs=[hbm] * 10,
        out_specs=pl.BlockSpec(memory_space=pltpu.VMEM),
        scratch_shapes=[
            pltpu.VMEM((1, D), BF16),
            pltpu.VMEM((1, D), BF16),
            pltpu.VMEM((F // LANE, LANE), BF16),
            pltpu.VMEM((D, 6 * D), BF16),
            pltpu.VMEM((D, H * DH), BF16),
            pltpu.VMEM((H * DH, D), BF16),
            pltpu.VMEM((D, F), BF16),
            pltpu.VMEM((F, D), BF16),
            pltpu.VMEM((NSLOT, window // LANE, PAIR, LANE), BF16),
            pltpu.VMEM((NSLOT, window // LANE, PAIR, LANE), BF16),
            pltpu.VMEM((NPAIR, 8, PAIR), F32),
            pltpu.VMEM((8, window), F32),
            pltpu.VMEM((8, D), F32),
            pltpu.VMEM((6, 8, D), F32),
            pltpu.VMEM((F, LANE), F32),
            pltpu.SemaphoreType.DMA((7 + len(W2_MXU) + len(W2_VPU),)),
            pltpu.SemaphoreType.DMA((2, NSLOT)),
            pltpu.SemaphoreType.REGULAR,
        ],
        compiler_params=pltpu.CompilerParams(
            vmem_limit_bytes=64 * 2**20,
            disable_semaphore_checks=True,
        ),
        name="adaln_attn_mlp_decode",
    )(A_x.reshape(1, D), _tiles(A_k_cache), _tiles(A_v_cache), A_wq, A_wo, B_w1,
      B_b1.reshape(F // LANE, LANE), B_w2, c, w_mod)
    return out.reshape(A_x.shape)
```

```python
import jax
import jax.numpy as jnp
from jax import lax
import jax.experimental.pallas as pl
import jax.experimental.pallas.tpu as pltpu

D = 640
H = 32
DH = 192
F = 1536
PAIR = 2 * DH
NPAIR = H // 2
SUB = 8
LANE = 128
PIECE = 8
F32 = jnp.float32
BF16 = jnp.bfloat16

NSLOT = 3
SHIFT = 4
QUEUE = (0, 1, 1, 1)
LAG = 25
LOOK = 80
W1_LOOK = 40
W2_LOOK = 35
PACE = 10
STEPS = 8
W2_LANES = 4
W2_MXU = (10, 10)
W2_VPU = (4, 3, 2, 1)


def _layernorm(x, eps=1e-5):
    m = jnp.mean(x, axis=-1, keepdims=True)
    d = x - m
    v = jnp.mean(d * d, axis=-1, keepdims=True)
    return d / jnp.sqrt(v + eps)


def _mish(u):
    softplus = jnp.log1p(jnp.exp(-jnp.abs(u))) + jnp.where(u > 0, u, 0.0)
    return u * jnp.tanh(softplus)


def _dot(a, b):
    return jnp.dot(a, b, preferred_element_type=F32)


class _Copy:
    def __init__(self, *refs):
        self.refs = refs

    def __call__(self, priority):
        pltpu.make_async_copy(*self.refs).start(priority=priority)

    def wait(self):
        pltpu.make_async_copy(*self.refs).wait()


def _num_pieces(ref):
    return ref.shape[0] * ref.shape[1] // (SUB * LANE * PIECE)


def _pieces(src, dst, sem, order):
    tiles = src.shape[1] // LANE
    out = []
    for q in order:
        t, end, rects = q * PIECE, (q + 1) * PIECE, []
        while t < end:
            r, c = divmod(t, tiles)
            n = min(tiles - c, end - t)
            idx = (pl.ds(r * SUB, SUB), pl.ds(c * LANE, n * LANE))
            rects.append(_Copy(src.at[idx], dst.at[idx], sem))
            t += n
        out.append(rects)
    return out


def _matrix(src, dst, sem, jump):
    n = _num_pieces(src)
    return _pieces(src, dst, sem, [q for first in range(jump) for q in range(first, n, jump)])


class _Stream:
    def __init__(self, parts, fence, pos=0):
        self.ends = []
        pieces = []
        for i, part in enumerate(parts):
            pieces += [(i, piece) for piece in part]
            self.ends.append(len(pieces))
        queue = [QUEUE[n % len(QUEUE)] for n in range(len(pieces))]
        late = [(cp, 1, i) for (i, piece), q in zip(pieces, queue) if q for cp in piece]
        self.slots, taken = [], LAG
        for (i, piece), q in zip(pieces, queue):
            if q:
                self.slots.append(late[taken:taken + len(piece)])
                taken += len(piece)
            else:
                self.slots.append([(cp, 0, i) for cp in piece])
        self.slots[0] = late[:LAG] + self.slots[0]
        self.fence = fence
        self.pos = pos
        self.part = None

    def upto(self, n):
        while self.pos < min(n, len(self.slots)):
            for cp, queue, part in self.slots[self.pos]:
                if self.part not in (None, part):
                    self.fence()
                self.part = part
                cp(queue)
            self.pos += 1

    def more(self, n):
        self.upto(self.pos + n)

    def past(self, part, look=LOOK):
        self.upto(self.ends[part] + look)


def _wait_all(buf, sem):
    pltpu.make_async_copy(buf, buf, sem).wait()


def _wait_pieces(pieces):
    for piece in pieces:
        for cp in piece:
            cp.wait()


def _kernel(x_hbm, k_hbm, v_hbm, wq_hbm, wo_hbm, w1_hbm, b1_hbm, w2_hbm, c_hbm, wmod_hbm, o_ref,
            x_v, c_v, b1_v, wmod_v, wq_v, wo_v, w1_v, w2_v, kbuf, vbuf, q_s, s_s, acc_s, mod_s, act_s,
            sem_w, sem_kv, sem_fence):
    nc = kbuf.shape[1]
    col0 = k_hbm.shape[1] - nc
    rows = PAIR // SUB
    half = rows * nc // PIECE

    def kv_piece(j, p, r, c):
        src, dst = ((k_hbm, kbuf), (v_hbm, vbuf))[j]

        def start(priority):
            slot = (p + r // rows) % NSLOT

            @pl.when(r < rows or p < NPAIR - 1)
            def _():
                pltpu.make_async_copy(
                    src.at[p * rows + r, pl.ds(col0 + c, PIECE)],
                    dst.at[slot, pl.ds(c, PIECE), pl.ds(r % rows * SUB, SUB), :],
                    sem_kv.at[j, slot]).start(priority=priority)

        return [start]

    def kv_pieces(j, p):
        return [kv_piece(j, p, r, c) for lo in (SHIFT, SHIFT + rows // 2)
                for first, way in ((lo, 1), (lo + 1, -1)) for c in range(0, nc, PIECE)[::way]
                for r in range(first, lo + rows // 2, 2)]

    def fence():
        pl.semaphore_signal(sem_fence, 1)
        pl.semaphore_wait(sem_fence, 1)

    s_c, s_x, s_b1, s_wmod, s_wq, s_wo, s_w1, s_w2 = range(8)

    head = _Stream([
        _matrix(wmod_hbm, wmod_v, sem_w.at[s_wmod], 32),
        _matrix(wq_hbm, wq_v, sem_w.at[s_wq], 64),
        _matrix(wo_hbm, wo_v, sem_w.at[s_wo], 64),
        *[[kv_piece(j, 0, r, c) for r in range(SHIFT)] for c in range(0, nc, PIECE) for j in range(2)],
        kv_pieces(0, 0), kv_pieces(1, 0)], fence)
    head.upto(1)
    small = [pltpu.make_async_copy(s, d, sem_w.at[i])
             for i, s, d in ((s_c, c_hbm, c_v), (s_x, x_hbm, x_v), (s_b1, b1_hbm, b1_v))]
    for cp in small:
        cp.start()
    head.past(0)
    for cp in small:
        cp.wait()
    _wait_all(wmod_v, sem_w.at[s_wmod])
    cf = c_v[...].astype(F32)
    silu_c = jnp.broadcast_to(cf * jax.nn.sigmoid(cf), (8, D)).astype(BF16)
    for i in range(6):
        mod_s[i] = _dot(silu_c, wmod_v[:, i * D:(i + 1) * D])
        head.more(48)
    x0 = jnp.broadcast_to(x_v[...].astype(F32), (8, D))
    h = (_layernorm(x0) * (1.0 + mod_s[1]) + mod_s[0]).astype(BF16)
    head.past(1)
    _wait_all(wq_v, sem_w.at[s_wq])
    row = lax.broadcasted_iota(jnp.int32, (8, PAIR), 0)
    col = lax.broadcasted_iota(jnp.int32, (8, PAIR), 1)
    own = jnp.logical_or(jnp.logical_and(row == 0, col < DH), jnp.logical_and(row == 1, col >= DH))
    for p in range(NPAIR):
        q_s[p] = jnp.where(own, _dot(h, wq_v[:, p * PAIR:(p + 1) * PAIR]), 0.0)
        head.more(24)
    head.past(2)
    _wait_all(wo_v, sem_w.at[s_wo])
    acc_s[...] = jnp.zeros(acc_s.shape, F32)
    head.past(-2)

    def scores(p, stream, step):
        slot = p % NSLOT
        _wait_all(kbuf.at[slot], sem_kv.at[0, slot])
        q = q_s[p].astype(BF16)
        for i in range(STEPS):
            for c in range(i * nc // STEPS, (i + 1) * nc // STEPS):
                s_s[:, c * LANE:(c + 1) * LANE] = _dot(q, kbuf[slot, c]) * DH ** -0.5
            stream.more(step)
        s = s_s[...]
        e = jnp.exp(s - jnp.max(s, axis=-1, keepdims=True))
        s_s[...] = e
        return jnp.sum(e, axis=-1, keepdims=True)

    def values(p, denom, stream, step):
        slot = p % NSLOT
        _wait_all(vbuf.at[slot], sem_kv.at[1, slot])
        o = jnp.zeros((8, PAIR), F32)
        for i in range(STEPS):
            for c in range(i * nc // STEPS, (i + 1) * nc // STEPS):
                o += lax.dot_general(s_s[:, c * LANE:(c + 1) * LANE].astype(BF16), vbuf[slot, c],
                                     (((1,), (1,)), ((), ())), preferred_element_type=F32)
            stream.more(step)
        o = jnp.where(own, o / denom, 0.0).astype(BF16)
        r0 = p * PAIR
        if not isinstance(r0, int):
            r0 = pl.multiple_of(r0, PAIR)
        acc_s[...] += _dot(o, wo_v[pl.ds(r0, PAIR), :])

    def body(p, carry):
        stream = _Stream([kv_pieces(1, p), kv_pieces(0, p + 1), kv_pieces(1, p + 1)], fence, LOOK)
        denom = scores(p, stream, half // (STEPS + 1))
        stream.past(0)
        values(p, denom, stream, half // (STEPS + 1))
        stream.past(1)
        return carry

    lax.fori_loop(0, NPAIR - 1, body, 0)

    per_lane = _num_pieces(w2_v) // W2_LANES
    groups, first = [], 0
    for n in W2_MXU + W2_VPU:
        groups.append([l * per_lane + q for q in range(first, first + n) for l in range(W2_LANES)])
        first += n
    assert first == per_lane
    w2_parts = [_pieces(w2_hbm, w2_v, sem_w.at[s_w2 + i], g) for i, g in enumerate(groups)]
    tail = _Stream([kv_pieces(1, NPAIR - 1), _matrix(w1_hbm, w1_v, sem_w.at[s_w1], 32),
                    [piece for part in w2_parts for piece in part]], fence, LOOK)
    denom = scores(NPAIR - 1, tail, (half - 20) // (STEPS + 1))
    tail.past(0, LOOK - 20)
    values(NPAIR - 1, denom, tail, PACE)

    att = jnp.broadcast_to(jnp.sum(acc_s[...], axis=0, keepdims=True), (8, D))
    x1 = x0 + mod_s[2] * att
    h2 = (_layernorm(x1) * (1.0 + mod_s[4]) + mod_s[3]).astype(BF16)
    b1 = b1_v[...].astype(F32)
    tail.past(1, W1_LOOK)
    _wait_all(w1_v, sem_w.at[s_w1])
    width = F // W2_LANES
    acts = []
    for c0 in range(0, F, width):
        bias = jnp.concatenate([jnp.broadcast_to(b1[t:t + 1, :], (8, LANE))
                                for t in range(c0 // LANE, (c0 + width) // LANE)], axis=1)
        acts.append(_mish(_dot(h2, w1_v[:, c0:c0 + width]) + bias).astype(BF16))
        tail.more(PACE)
    act = jnp.concatenate(acts, axis=1)
    for l in range(W2_LANES):
        for c0 in range(l * width + len(W2_MXU) * LANE, (l + 1) * width, LANE):
            act_s[c0:c0 + LANE, :] = jnp.broadcast_to(act[:1, c0:c0 + LANE].astype(F32), (LANE, LANE)).T

    y = jnp.zeros((8, D), F32)
    done = tail.ends[1]
    for i in range(len(W2_MXU)):
        done += len(groups[i])
        tail.upto(done + W2_LOOK)
        _wait_pieces(w2_parts[i])
        for r in range(i * LANE, F, width):
            y += _dot(act[:, r:r + LANE], w2_v[r:r + LANE, :])
            acc_s[...] = y
            tail.more(2)
    tail.past(2)
    gate = mod_s[5]
    partial = x1 + gate * y
    acc = [jnp.zeros((SUB, LANE), F32)] * (D // LANE)
    for i in range(len(W2_MXU), len(groups)):
        _wait_pieces(w2_parts[i])
        for q in groups[i]:
            for t in range(q * PIECE, (q + 1) * PIECE):
                r, c = divmod(t, D // LANE)
                w = w2_v[r * SUB:(r + 1) * SUB, c * LANE:(c + 1) * LANE].astype(F32)
                acc[c] = acc[c] + w * act_s[r * SUB:(r + 1) * SUB, :]
        acc_s[...] = jnp.concatenate(acc, axis=1)
    y = jnp.sum(jnp.concatenate(acc, axis=1), axis=0, keepdims=True)
    o_ref[...] = (partial[0:1] + gate[0:1] * y).astype(o_ref.dtype)


def _tiles(cache):
    t = jnp.swapaxes(cache, 2, 3).reshape(H * DH // SUB, SUB, cache.shape[2] // LANE, LANE)
    return t.transpose(0, 2, 1, 3)


@jax.jit
def pallas_adaLN_cond__sliding_block_cached__dense_activation_mish__decode_kernel(
    A_x: jax.Array,
    A_k_cache: jax.Array,
    A_v_cache: jax.Array,
    A_wq: jax.Array,
    A_wo: jax.Array,
    B_x: jax.Array,
    B_w1: jax.Array,
    B_b1: jax.Array,
    B_w2: jax.Array,
    c: jax.Array,
    w_mod: jax.Array,
):
    del B_x
    window = min(4096, max(256, A_k_cache.shape[2] // 4))
    hbm = pl.BlockSpec(memory_space=pltpu.HBM)
    out = pl.pallas_call(
        _kernel,
        out_shape=jax.ShapeDtypeStruct((1, D), A_x.dtype),
        in_specs=[hbm] * 10,
        out_specs=pl.BlockSpec(memory_space=pltpu.VMEM),
        scratch_shapes=[
            pltpu.VMEM((1, D), BF16),
            pltpu.VMEM((1, D), BF16),
            pltpu.VMEM((F // LANE, LANE), BF16),
            pltpu.VMEM((D, 6 * D), BF16),
            pltpu.VMEM((D, H * DH), BF16),
            pltpu.VMEM((H * DH, D), BF16),
            pltpu.VMEM((D, F), BF16),
            pltpu.VMEM((F, D), BF16),
            pltpu.VMEM((NSLOT, window // LANE, PAIR, LANE), BF16),
            pltpu.VMEM((NSLOT, window // LANE, PAIR, LANE), BF16),
            pltpu.VMEM((NPAIR, 8, PAIR), F32),
            pltpu.VMEM((8, window), F32),
            pltpu.VMEM((8, D), F32),
            pltpu.VMEM((6, 8, D), F32),
            pltpu.VMEM((F, LANE), F32),
            pltpu.SemaphoreType.DMA((7 + len(W2_MXU) + len(W2_VPU),)),
            pltpu.SemaphoreType.DMA((2, NSLOT)),
            pltpu.SemaphoreType.REGULAR,
        ],
        compiler_params=pltpu.CompilerParams(
            vmem_limit_bytes=64 * 2**20,
            disable_semaphore_checks=True,
        ),
        name="adaln_attn_mlp_decode",
    )(A_x.reshape(1, D), _tiles(A_k_cache), _tiles(A_v_cache), A_wq, A_wo, B_w1,
      B_b1.reshape(F // LANE, LANE), B_w2, c, w_mod)
    return out.reshape(A_x.shape)
```

```python
import jax
import jax.numpy as jnp
from jax import lax
import jax.experimental.pallas as pl
import jax.experimental.pallas.tpu as pltpu

D = 640
H = 32
DH = 192
F = 1536
PAIR = 2 * DH
NPAIR = H // 2
SUB = 8
LANE = 128
PIECE = 8
F32 = jnp.float32
BF16 = jnp.bfloat16

NSLOT = 3
SHIFT = 4
QUEUE = (0, 1, 1, 1)
LAG = 26
LOOK = 80
W1_LOOK = 36
W2_LOOK = 30
PACE = 10
STEPS = 8
W2_LANES = 4
W2_MXU = (10, 10)
W2_VPU = (4, 3, 2, 1)


def _layernorm(x, eps=1e-5):
    m = jnp.mean(x, axis=-1, keepdims=True)
    d = x - m
    v = jnp.mean(d * d, axis=-1, keepdims=True)
    return d / jnp.sqrt(v + eps)


def _mish(u):
    softplus = jnp.log1p(jnp.exp(-jnp.abs(u))) + jnp.where(u > 0, u, 0.0)
    return u * jnp.tanh(softplus)


def _dot(a, b):
    return jnp.dot(a, b, preferred_element_type=F32)


class _Copy:
    def __init__(self, *refs):
        self.refs = refs

    def __call__(self, priority):
        pltpu.make_async_copy(*self.refs).start(priority=priority)

    def wait(self):
        pltpu.make_async_copy(*self.refs).wait()


def _num_pieces(ref):
    return ref.shape[0] * ref.shape[1] // (SUB * LANE * PIECE)


def _pieces(src, dst, sem, order):
    tiles = src.shape[1] // LANE
    out = []
    for q in order:
        t, end, rects = q * PIECE, (q + 1) * PIECE, []
        while t < end:
            r, c = divmod(t, tiles)
            n = min(tiles - c, end - t)
            idx = (pl.ds(r * SUB, SUB), pl.ds(c * LANE, n * LANE))
            rects.append(_Copy(src.at[idx], dst.at[idx], sem))
            t += n
        out.append(rects)
    return out


def _matrix(src, dst, sem, jump):
    n = _num_pieces(src)
    return _pieces(src, dst, sem, [q for first in range(jump) for q in range(first, n, jump)])


class _Stream:
    def __init__(self, parts, fence, pos=0):
        self.ends = []
        pieces = []
        for i, part in enumerate(parts):
            assert len(part) % len(QUEUE) == 0
            pieces += [(i, piece) for piece in part]
            self.ends.append(len(pieces))
        queue = [QUEUE[n % len(QUEUE)] for n in range(len(pieces))]
        late = [(cp, 1, i) for (i, piece), q in zip(pieces, queue) if q for cp in piece]
        self.slots, taken = [], LAG
        for (i, piece), q in zip(pieces, queue):
            if q:
                self.slots.append(late[taken:taken + len(piece)])
                taken += len(piece)
            else:
                self.slots.append([(cp, 0, i) for cp in piece])
        self.slots[0] = late[:LAG] + self.slots[0]
        self.fence = fence
        self.pos = pos
        self.part = None

    def upto(self, n):
        while self.pos < min(n, len(self.slots)):
            for cp, queue, part in self.slots[self.pos]:
                if self.part not in (None, part):
                    self.fence()
                self.part = part
                cp(queue)
            self.pos += 1

    def more(self, n):
        self.upto(self.pos + n)

    def past(self, part, look=LOOK):
        self.upto(self.ends[part] + look)


def _wait_all(buf, sem):
    pltpu.make_async_copy(buf, buf, sem).wait()


def _wait_pieces(pieces):
    for piece in pieces:
        for cp in piece:
            cp.wait()


def _kernel(x_hbm, k_hbm, v_hbm, wq_hbm, wo_hbm, w1_hbm, b1_hbm, w2_hbm, c_hbm, wmod_hbm, o_ref,
            x_v, c_v, b1_v, wmod_v, wq_v, wo_v, w1_v, w2_v, kbuf, vbuf, q_s, s_s, acc_s, mod_s, act_s,
            sem_w, sem_kv, sem_fence):
    nc = kbuf.shape[1]
    col0 = k_hbm.shape[1] - nc
    rows = PAIR // SUB
    half = rows * nc // PIECE

    def kv_piece(j, p, r, c):
        src, dst = ((k_hbm, kbuf), (v_hbm, vbuf))[j]

        def start(priority):
            slot = (p + r // rows) % NSLOT

            @pl.when(r < rows or p < NPAIR - 1)
            def _():
                pltpu.make_async_copy(
                    src.at[p * rows + r, pl.ds(col0 + c, PIECE)],
                    dst.at[slot, pl.ds(c, PIECE), pl.ds(r % rows * SUB, SUB), :],
                    sem_kv.at[j, slot]).start(priority=priority)

        return [start]

    def kv_pieces(j, p):
        return [kv_piece(j, p, r, c) for lo in (SHIFT, SHIFT + rows // 2)
                for first, way in ((lo, 1), (lo + 1, -1)) for c in range(0, nc, PIECE)[::way]
                for r in range(first, lo + rows // 2, 2)]

    def fence():
        pl.semaphore_signal(sem_fence, 1)
        pl.semaphore_wait(sem_fence, 1)

    s_c, s_x, s_b1, s_wmod, s_wq, s_wo, s_w1, s_w2 = range(8)

    head = _Stream([
        _matrix(wmod_hbm, wmod_v, sem_w.at[s_wmod], 32),
        _matrix(wq_hbm, wq_v, sem_w.at[s_wq], 64),
        _matrix(wo_hbm, wo_v, sem_w.at[s_wo], 64),
        *[[kv_piece(j, 0, r, c) for r in range(SHIFT)] for c in range(0, nc, PIECE) for j in range(2)],
        kv_pieces(0, 0), kv_pieces(1, 0)], fence)
    head.upto(1)
    small = [pltpu.make_async_copy(s, d, sem_w.at[i])
             for i, s, d in ((s_c, c_hbm, c_v), (s_x, x_hbm, x_v), (s_b1, b1_hbm, b1_v))]
    for cp in small:
        cp.start()
    head.past(0)
    for cp in small:
        cp.wait()
    _wait_all(wmod_v, sem_w.at[s_wmod])
    cf = c_v[...].astype(F32)
    silu_c = jnp.broadcast_to(cf * jax.nn.sigmoid(cf), (8, D)).astype(BF16)
    for i in range(6):
        mod_s[i] = _dot(silu_c, wmod_v[:, i * D:(i + 1) * D])
        head.more(48)
    x0 = jnp.broadcast_to(x_v[...].astype(F32), (8, D))
    h = (_layernorm(x0) * (1.0 + mod_s[1]) + mod_s[0]).astype(BF16)
    head.past(1)
    _wait_all(wq_v, sem_w.at[s_wq])
    row = lax.broadcasted_iota(jnp.int32, (8, PAIR), 0)
    col = lax.broadcasted_iota(jnp.int32, (8, PAIR), 1)
    own = jnp.logical_or(jnp.logical_and(row == 0, col < DH), jnp.logical_and(row == 1, col >= DH))
    for p in range(NPAIR):
        q_s[p] = jnp.where(own, _dot(h, wq_v[:, p * PAIR:(p + 1) * PAIR]), 0.0)
        head.more(24)
    head.past(2)
    _wait_all(wo_v, sem_w.at[s_wo])
    acc_s[...] = jnp.zeros(acc_s.shape, F32)
    head.past(-2)

    def scores(p, stream, step):
        slot = p % NSLOT
        _wait_all(kbuf.at[slot], sem_kv.at[0, slot])
        q = q_s[p].astype(BF16)
        for i in range(STEPS):
            for c in range(i * nc // STEPS, (i + 1) * nc // STEPS):
                s_s[:, c * LANE:(c + 1) * LANE] = _dot(q, kbuf[slot, c]) * DH ** -0.5
            stream.more(step)
        s = s_s[...]
        e = jnp.exp(s - jnp.max(s, axis=-1, keepdims=True))
        s_s[...] = e
        return jnp.sum(e, axis=-1, keepdims=True)

    def values(p, denom, stream, step):
        slot = p % NSLOT
        _wait_all(vbuf.at[slot], sem_kv.at[1, slot])
        o = jnp.zeros((8, PAIR), F32)
        for i in range(STEPS):
            for c in range(i * nc // STEPS, (i + 1) * nc // STEPS):
                o += lax.dot_general(s_s[:, c * LANE:(c + 1) * LANE].astype(BF16), vbuf[slot, c],
                                     (((1,), (1,)), ((), ())), preferred_element_type=F32)
            stream.more(step)
        o = jnp.where(own, o / denom, 0.0).astype(BF16)
        r0 = p * PAIR
        if not isinstance(r0, int):
            r0 = pl.multiple_of(r0, PAIR)
        acc_s[...] += _dot(o, wo_v[pl.ds(r0, PAIR), :])

    def body(p, carry):
        stream = _Stream([kv_pieces(1, p), kv_pieces(0, p + 1), kv_pieces(1, p + 1)], fence, LOOK)
        denom = scores(p, stream, half // (STEPS + 1))
        stream.past(0)
        values(p, denom, stream, half // (STEPS + 1))
        stream.past(1)
        return carry

    lax.fori_loop(0, NPAIR - 1, body, 0)

    per_lane = _num_pieces(w2_v) // W2_LANES
    groups, first = [], 0
    for n in W2_MXU + W2_VPU:
        groups.append([l * per_lane + q for q in range(first, first + n) for l in range(W2_LANES)])
        first += n
    assert first == per_lane
    w2_parts = [_pieces(w2_hbm, w2_v, sem_w.at[s_w2 + i], g) for i, g in enumerate(groups)]
    tail = _Stream([kv_pieces(1, NPAIR - 1), _matrix(w1_hbm, w1_v, sem_w.at[s_w1], 32),
                    [piece for part in w2_parts for piece in part]], fence, LOOK)
    denom = scores(NPAIR - 1, tail, (half - 20) // (STEPS + 1))
    tail.past(0, LOOK - 20)
    values(NPAIR - 1, denom, tail, PACE)

    att = jnp.broadcast_to(jnp.sum(acc_s[...], axis=0, keepdims=True), (8, D))
    x1 = x0 + mod_s[2] * att
    h2 = (_layernorm(x1) * (1.0 + mod_s[4]) + mod_s[3]).astype(BF16)
    b1 = b1_v[...].astype(F32)
    tail.past(1, W1_LOOK)
    _wait_all(w1_v, sem_w.at[s_w1])
    width = F // W2_LANES
    acts = []
    for c0 in range(0, F, width):
        bias = jnp.concatenate([jnp.broadcast_to(b1[t:t + 1, :], (8, LANE))
                                for t in range(c0 // LANE, (c0 + width) // LANE)], axis=1)
        acts.append(_mish(_dot(h2, w1_v[:, c0:c0 + width]) + bias).astype(BF16))
        tail.more(PACE)
    act = jnp.concatenate(acts, axis=1)
    for l in range(W2_LANES):
        for c0 in range(l * width + len(W2_MXU) * LANE, (l + 1) * width, LANE):
            act_s[c0:c0 + LANE, :] = jnp.broadcast_to(act[:1, c0:c0 + LANE].astype(F32), (LANE, LANE)).T

    y = jnp.zeros((8, D), F32)
    done = tail.ends[1]
    for i in range(len(W2_MXU)):
        done += len(groups[i])
        tail.upto(done + W2_LOOK)
        _wait_pieces(w2_parts[i])
        for r in range(i * LANE, F, width):
            y += _dot(act[:, r:r + LANE], w2_v[r:r + LANE, :])
            acc_s[...] = y
            tail.more(2)
    tail.past(2)
    gate = mod_s[5]
    partial = x1 + gate * y
    acc = [jnp.zeros((SUB, LANE), F32)] * (D // LANE)
    for i in range(len(W2_MXU), len(groups)):
        _wait_pieces(w2_parts[i])
        for q in groups[i]:
            for t in range(q * PIECE, (q + 1) * PIECE):
                r, c = divmod(t, D // LANE)
                w = w2_v[r * SUB:(r + 1) * SUB, c * LANE:(c + 1) * LANE].astype(F32)
                acc[c] = acc[c] + w * act_s[r * SUB:(r + 1) * SUB, :]
        acc_s[...] = jnp.concatenate(acc, axis=1)
    y = jnp.sum(jnp.concatenate(acc, axis=1), axis=0, keepdims=True)
    o_ref[...] = (partial[0:1] + gate[0:1] * y).astype(o_ref.dtype)


def _tiles(cache):
    t = jnp.swapaxes(cache, 2, 3).reshape(H * DH // SUB, SUB, cache.shape[2] // LANE, LANE)
    return t.transpose(0, 2, 1, 3)


@jax.jit
def pallas_adaLN_cond__sliding_block_cached__dense_activation_mish__decode_kernel(
    A_x: jax.Array,
    A_k_cache: jax.Array,
    A_v_cache: jax.Array,
    A_wq: jax.Array,
    A_wo: jax.Array,
    B_x: jax.Array,
    B_w1: jax.Array,
    B_b1: jax.Array,
    B_w2: jax.Array,
    c: jax.Array,
    w_mod: jax.Array,
):
    del B_x
    window = min(4096, max(256, A_k_cache.shape[2] // 4))
    hbm = pl.BlockSpec(memory_space=pltpu.HBM)
    out = pl.pallas_call(
        _kernel,
        out_shape=jax.ShapeDtypeStruct((1, D), A_x.dtype),
        in_specs=[hbm] * 10,
        out_specs=pl.BlockSpec(memory_space=pltpu.VMEM),
        scratch_shapes=[
            pltpu.VMEM((1, D), BF16),
            pltpu.VMEM((1, D), BF16),
            pltpu.VMEM((F // LANE, LANE), BF16),
            pltpu.VMEM((D, 6 * D), BF16),
            pltpu.VMEM((D, H * DH), BF16),
            pltpu.VMEM((H * DH, D), BF16),
            pltpu.VMEM((D, F), BF16),
            pltpu.VMEM((F, D), BF16),
            pltpu.VMEM((NSLOT, window // LANE, PAIR, LANE), BF16),
            pltpu.VMEM((NSLOT, window // LANE, PAIR, LANE), BF16),
            pltpu.VMEM((NPAIR, 8, PAIR), F32),
            pltpu.VMEM((8, window), F32),
            pltpu.VMEM((8, D), F32),
            pltpu.VMEM((6, 8, D), F32),
            pltpu.VMEM((F, LANE), F32),
            pltpu.SemaphoreType.DMA((7 + len(W2_MXU) + len(W2_VPU),)),
            pltpu.SemaphoreType.DMA((2, NSLOT)),
            pltpu.SemaphoreType.REGULAR,
        ],
        compiler_params=pltpu.CompilerParams(
            vmem_limit_bytes=64 * 2**20,
            disable_semaphore_checks=True,
        ),
        name="adaln_attn_mlp_decode",
    )(A_x.reshape(1, D), _tiles(A_k_cache), _tiles(A_v_cache), A_wq, A_wo, B_w1,
      B_b1.reshape(F // LANE, LANE), B_w2, c, w_mod)
    return out.reshape(A_x.shape)
```
